```python
import os as _os
_os.environ.setdefault("JAX_PLATFORMS", "cpu")
import jax
import jax.numpy as jnp

def _softmax(x, axis=-1):
    return jax.nn.softmax(x, axis=axis)
def _gelu(x):
    return jax.nn.gelu(x, approximate=True)
def _silu(x):
    return jax.nn.silu(x)
def _sigmoid(x):
    return jax.nn.sigmoid(x)
def _layernorm(x, axis=-1, eps=1e-5):
    m = jnp.mean(x, axis=axis, keepdims=True)
    v = jnp.var(x, axis=axis, keepdims=True)
    return (x - m) / jnp.sqrt(v + eps)
def _scatter_add(tgt, idx, src, axis=0):
    return tgt.at[idx].add(src)
def _segment_sum(src, seg, n):
    return jax.ops.segment_sum(src, seg, n)
class _Rng:
    def __init__(self, key):
        self._k = key
    def _next(self):
        self._k, sub = jax.random.split(self._k)
        return sub
    def normal(self, shape):
        return jax.random.normal(self._next(), shape, dtype=jnp.bfloat16)
    def randint(self, lo, hi, shape):
        return jax.random.randint(self._next(), shape, lo, hi, dtype=jnp.int32)
    def uniform(self, shape, lo=0.0, hi=1.0):
        return jax.random.uniform(self._next(), shape, jnp.bfloat16, lo, hi)
    def permutation(self, n):
        return jax.random.permutation(self._next(), n)


kernel_name = 'gated_mix__ssm_conv_s5__glu_gated_geglu__prompt'

def setup_inputs():
    _rng = _Rng(jax.random.key(int.from_bytes(__import__("os").urandom(4), "little")))
    _w = (lambda a: (lambda t: t.astype(jnp.bfloat16) if jnp.issubdtype(t.dtype, jnp.floating) else t)(jnp.asarray(a)))
    def _A_setup():
        B, S, D = 1, 2048, 448
        P = D
        Lambda_re = -0.5 * jnp.exp((lambda *s: _rng.normal(s) * 0.4)(P))
        Lambda_im = (lambda *s: _rng.normal(s) * 0.4)(P) * 1.0
        B_re = (lambda *s: _rng.normal(s) * 0.4)(P, D) * (D ** -0.5)
        B_im = (lambda *s: _rng.normal(s) * 0.4)(P, D) * (D ** -0.5)
        C_re = (lambda *s: _rng.normal(s) * 0.4)(D, P) * (P ** -0.5)
        C_im = (lambda *s: _rng.normal(s) * 0.4)(D, P) * (P ** -0.5)
        log_dt = (lambda *s: _rng.normal(s) * 0.4)(P) * 0.3 - 2.0
        Dskip = (lambda *s: _rng.normal(s) * 0.4)(D)
        return {
            "x": _w((lambda *s: _rng.normal(s) * 0.05)(B, S, D)),
            "Lambda_re": _w(Lambda_re),
            "Lambda_im": _w(Lambda_im),
            "B_re": _w(B_re),
            "B_im": _w(B_im),
            "C_re": _w(C_re),
            "C_im": _w(C_im),
            "log_dt": _w(log_dt),
            "Dskip": _w(Dskip),
        }
    _A_in = _A_setup()

    def _B_setup():
        B, S, Dm, Df = 1, 2048, 448, 1792
        return {
            "x": _w((lambda *s: _rng.normal(s) * 0.05)(B, S, Dm)),
            "w_gate": _w((lambda *s: _rng.normal(s) * 1.6)(Dm, Df) * (Dm ** -0.5)),
            "w_up": _w((lambda *s: _rng.normal(s) * 1.6)(Dm, Df) * (Dm ** -0.5)),
            "w_down": _w((lambda *s: _rng.normal(s) * 1.6)(Df, Dm) * (Df ** -0.5)),
        }
    _B_in = _B_setup()

    return {
        "A_x": _A_in["x"],
        "A_Lambda_re": _A_in["Lambda_re"],
        "A_Lambda_im": _A_in["Lambda_im"],
        "A_B_re": _A_in["B_re"],
        "A_B_im": _A_in["B_im"],
        "A_C_re": _A_in["C_re"],
        "A_C_im": _A_in["C_im"],
        "A_log_dt": _A_in["log_dt"],
        "A_Dskip": _A_in["Dskip"],
        "B_x": _B_in["x"],
        "B_w_gate": _B_in["w_gate"],
        "B_w_up": _B_in["w_up"],
        "B_w_down": _B_in["w_down"],
        "gate_w": _w((lambda *s: _rng.normal(s) * 0.05)(448) * 16.0),
    }

def reference(A_x, A_Lambda_re, A_Lambda_im, A_B_re, A_B_im, A_C_re, A_C_im, A_log_dt, A_Dskip, B_x, B_w_gate, B_w_up, B_w_down, gate_w):
    def _A_ref(x, Lambda_re, Lambda_im, B_re, B_im, C_re, C_im, log_dt, Dskip):
        Bsz, L, H = x.shape
        Lam = Lambda_re + 1j * Lambda_im
        Bmat = B_re + 1j * B_im
        Cmat = C_re + 1j * C_im
        dt = jnp.exp(log_dt)
        Lam_bar = jnp.exp(dt * Lam)
        B_bar = ((Lam_bar - 1.0) / Lam)[:, None] * Bmat
        Bu = jnp.einsum("bld,pd->blp", x + 0j, B_bar)
        h = jnp.zeros_like(Bu[:, 0, :])
        hs = []
        for t in range(L):
            h = Lam_bar[None, :] * h + Bu[:, t, :]
            hs.append(h)
        hseq = jnp.stack(hs, 1)
        y = 2.0 * jnp.einsum("blp,dp->bld", hseq, Cmat).real + x * Dskip[None, None, :]
        return y

    def _B_ref(x, w_gate, w_up, w_down):
        g = jnp.einsum("bsd,df->bsf", x, w_gate)
        u = jnp.einsum("bsd,df->bsf", x, w_up)
        h = _gelu(g) * u
        return jnp.einsum("bsf,fd->bsd", h, w_down)

    x = A_x
    g = _sigmoid((x * gate_w).sum(-1, keepdims=True))
    a = _A_ref(x, A_Lambda_re, A_Lambda_im, A_B_re, A_B_im, A_C_re, A_C_im, A_log_dt, A_Dskip)
    b = _B_ref(x, B_w_gate, B_w_up, B_w_down)
    return g * a + (1 - g) * b
```

```python
import jax
import jax.numpy as jnp
import numpy as np
from jax import lax
import jax.experimental.pallas as pl
import jax.experimental.pallas.tpu as pltpu

bf = jnp.bfloat16
f32 = jnp.float32
u32 = jnp.uint32
i32 = jnp.int32

D = 448
P = 448
F = 1792
M = 2048
NT = M // 128


def nn(a, b):
    return jnp.dot(a, b, preferred_element_type=f32)


def nt(a, b):
    return lax.dot_general(a, b, (((1,), (1,)), ((), ())), preferred_element_type=f32)


def tobf(v):
    return pltpu.bitcast(v, bf)


def tou(v):
    return pltpu.bitcast(v, u32)


def cmul(ar, ai, br, bi):
    return ar * br - ai * bi, ar * bi + ai * br


def cmac(ar, ai, br, bi, cr, ci):
    return (ar * br - ai * bi) + cr, (ar * bi + ai * br) + ci


def make(OPT=None):
    OPT = dict(OPT or {})
    PACE = OPT.get("pace", True)
    SCAN_LEAD = OPT.get("scan_lead", 1)
    R1A = OPT.get("r1a", 128)
    R1B = OPT.get("r1b", 256)
    KB = OPT.get("kb", 4)
    P1_SCAN_TILES = OPT.get("p1_scan_tiles", 3)
    P1_SCAN_RATE = OPT.get("p1_scan_rate", 3)
    P2_RATE_A = OPT.get("p2a", 3)
    P2_RATE_B = OPT.get("p2b", 2)
    LEAD = OPT.get("lead", 2)
    DEP_BOTH = OPT.get("dep_both", True)
    ANC_ROW = OPT.get("anc_row", 0)
    WG_AT = OPT.get("wg_at", 8)
    WU_AT = OPT.get("wu_at", 12)

    def kernel(xT, lre_h, lim_h, bre, bim, cre, cim, ldt_h, dsk_h, wg, wu, wdT, gw_h, o_hbm,
               lre_v, lim_v, ldt_v, dsk_v, gw_v,
               xn, Bk, Bt, wgr, wur, crr, cir, Wk32, Wt32, W2A, W2B, tabs, ltab, b, HA, HB, ob,
               sem, osem):
        xn32 = xn.bitcast(u32)
        Bk32 = Bk.bitcast(u32)
        Bt32 = Bt.bitcast(u32)
        W2A32 = W2A.bitcast(u32)
        W2B32 = W2B.bitcast(u32)
        HA32 = HA.bitcast(u32)
        HB32 = HB.bitcast(u32)

        lane = lax.broadcasted_iota(i32, (8, 128), 1)
        sub = lax.broadcasted_iota(i32, (8, 128), 0)
        zero_u = (lane >> 8).astype(u32)

        nsem = [0]

        def cp(src, dst):
            c = pltpu.make_async_copy(src, dst, sem.at[nsem[0]])
            nsem[0] += 1
            return c

        cvec = [cp(lre_h, lre_v), cp(lim_h, lim_v), cp(ldt_h, ldt_v), cp(dsk_h, dsk_v), cp(gw_h, gw_v)]
        cx = [cp(xT.at[:, pl.ds(j * 128, 128)], xn.at[j]) for j in range(NT)]
        cB = []
        for ri, src in enumerate((bre, bim)):
            for k in range(3):
                cB.append(cp(src.at[:, pl.ds(k * 128, 128)], Bk.at[k, pl.ds(ri * P, P), :]))
            cB.append(cp(src.at[:, pl.ds(384, 64)], Bt.at[pl.ds(ri * P, P), :]))
        cwg = cp(wg, wgr)
        cwu = cp(wu, wur)
        cC = [cp(cre, crr), cp(cim, cir)]
        cwd = [cp(wdT.at[:, pl.ds(n * 128, 128)], W2B.at[n]) for n in range(14)]
        co = [pltpu.make_async_copy(ob.at[j], o_hbm.at[:, pl.ds(j * 128, 128)], osem.at[j]) for j in range(NT)]

        cx[0].start()
        for c in cB:
            c.start()
        for c in cvec:
            c.start()
        for j in range(1, 8):
            cx[j].start()
        cwg.start()
        for j in range(8, 12):
            cx[j].start()
        cwu.start()
        for j in range(12, 16):
            cx[j].start()
        for c in cC:
            c.start()
        for c in cwd:
            c.start()

        def ktile(ref32, t, k):
            if k < 3:
                return tobf(ref32[t, pl.ds(k * 64, 64), :])
            return tobf(ref32[t, pl.ds(192, 32), :])

        def s1a_chunks(t):
            for r0 in range(0, 2 * P, R1A):
                acc = nn(tobf(Bt32[r0 // 2:(r0 + R1A) // 2, :]), ktile(xn32, t, 3))
                for k in range(3):
                    acc = acc + nn(tobf(Bk32[k, r0 // 2:(r0 + R1A) // 2, :]), ktile(xn32, t, k))
                b[t, pl.ds(r0, R1A), :] = acc
                yield acc[0:8, :]

        def row(ref):
            return ref[...].astype(f32).reshape(1, D)

        def to_col(slot, v):
            for n in range(4):
                w = 128 if n < 3 else 64
                tabs[slot, pl.ds(n * 128, w), :] = jnp.broadcast_to(v[:, n * 128:n * 128 + w], (128, w)).T

        coefs = {}

        def build_tables():
            lr = row(lre_v)
            li = row(lim_v)
            dt = jnp.exp(row(ldt_v)).astype(bf).astype(f32)
            mag = jnp.exp(dt * lr)
            th = dt * li
            lam_r = mag * jnp.cos(th)
            lam_i = mag * jnp.sin(th)
            nr = lam_r - 1.0
            ni = lam_i
            big = jnp.abs(lr) >= jnp.abs(li)
            ratio = jnp.where(big, li / lr, lr / li)
            den = jnp.where(big, lr + li * ratio, lr * ratio + li)
            coefs["r"] = jnp.where(big, nr + ni * ratio, nr * ratio + ni) / den
            coefs["i"] = jnp.where(big, ni - nr * ratio, ni * ratio - nr) / den
            to_col(0, row(dsk_v))
            to_col(1, row(gw_v))
            p1 = (jnp.broadcast_to(lam_r, (8, D)), jnp.broadcast_to(lam_i, (8, D)))
            p2 = cmul(*p1, *p1)
            p3 = cmul(*p2, *p1)
            p4 = cmul(*p2, *p2)
            p5 = cmul(*p4, *p1)
            p6 = cmul(*p4, *p2)
            p7 = cmul(*p4, *p3)
            p8 = cmul(*p4, *p4)
            pw = [p1, p2, p3, p4, p5, p6, p7, p8]
            s8 = lax.broadcasted_iota(i32, (8, D), 0)
            l8r, l8i = pw[7]
            for s in range(7):
                l8r = jnp.where(s8 == s, pw[s][0], l8r)
                l8i = jnp.where(s8 == s, pw[s][1], l8i)
            items = [jnp.where(s8 >= 1, p1[0], 0.0), jnp.where(s8 >= 1, p1[1], 0.0),
                     jnp.where(s8 >= 2, p2[0], 0.0), jnp.where(s8 >= 2, p2[1], 0.0),
                     jnp.where(s8 >= 4, p4[0], 0.0), jnp.where(s8 >= 4, p4[1], 0.0),
                     l8r, l8i]
            for q, it in enumerate(items):
                for n in range(3):
                    ltab[q, n] = it[:, n * 128:(n + 1) * 128]
                ltab[q, 3, :, pl.ds(0, 64)] = it[:, 384:448]

        def transposes(raw, which):
            for n in range(F // 128):
                for k in range(3):
                    v = tou(raw[pl.ds(k * 128, 128), pl.ds(n * 128, 128)].T)
                    Wk32[k, pl.ds(8 * n, 8), which] = v.reshape(8, 8, 128) | zero_u
                v = tou(raw[pl.ds(384, 64), pl.ds(n * 128, 128)].T)
                Wt32[pl.ds(8 * n, 8), which] = v.reshape(8, 8, 64) | zero_u[:, :64]

        def build_c():
            cr2 = coefs["r"] * 2.0
            ci2 = coefs["i"] * 2.0
            for r in range(D // 16):
                rows = pl.ds(16 * r, 16)
                tails = []
                for m in range(4):
                    w = 128 if m < 3 else 64
                    vr = crr[rows, pl.ds(m * 128, w)].astype(f32)
                    vi = cir[rows, pl.ds(m * 128, w)].astype(f32)
                    ar = cr2[:, m * 128:m * 128 + w]
                    ai = ci2[:, m * 128:m * 128 + w]
                    are = vr * ar - vi * ai
                    aim = -(vr * ai + vi * ar)
                    if m < 3:
                        W2A[m, rows, :] = are.astype(bf)
                        W2A[4 + m, rows, :] = aim.astype(bf)
                    else:
                        W2A[3, rows, :] = jnp.concatenate([are, aim], axis=1).astype(bf)

        carry = {}
        anc = {"a": None}

        def set_anchor(v):
            anc["a"] = None if v is None else (pltpu.bitcast(v, u32) & zero_u)

        def dep(v):
            a = anc["a"]
            if a is None:
                return v
            if v.shape[1] != 128:
                a = a[:, :v.shape[1]]
            return pltpu.bitcast(pltpu.bitcast(v, u32) | a, f32)

        def pace(v, anchor):
            if anchor is None:
                return v
            a = pltpu.bitcast(anchor, u32) & zero_u
            if v.shape[1] != 128:
                a = a[:, :v.shape[1]]
            return pltpu.bitcast(pltpu.bitcast(v, u32) | a, f32)

        def scan_steps(t):
            def tr(n):
                w = 128 if n < 3 else 64
                return (b[t, pl.ds(128 * n, w), :].T, b[t, pl.ds(P + 128 * n, w), :].T)
            nxt = tr(0)
            for n in range(4):
                w = 128 if n < 3 else 64
                tre, tim = nxt
                if n < 3:
                    nxt = tr(n + 1)
                if n < 3:
                    lt = [ltab[q, n] for q in range(8)]
                else:
                    lt = [ltab[q, 3, :, pl.ds(0, 64)] for q in range(8)]
                prev = None
                for v in range(16):
                    br = dep(tre[8 * v:8 * v + 8, :])
                    bi = dep(tim[8 * v:8 * v + 8, :]) if DEP_BOTH else tim[8 * v:8 * v + 8, :]
                    for q, sh in enumerate((1, 2, 4)):
                        sr = pltpu.roll(br, sh, 0)
                        si = pltpu.roll(bi, sh, 0)
                        br, bi = cmac(lt[2 * q], lt[2 * q + 1], sr, si, br, bi)
                    if t == 0 and v == 0:
                        hr, hi = br, bi
                    else:
                        cr, ci = carry[n]
                        hr, hi = cmac(lt[6], lt[7], cr, ci, br, bi)
                    carry[n] = (jnp.broadcast_to(hr[7:8, :], (8, w)), jnp.broadcast_to(hi[7:8, :], (8, w)))
                    if v % 2 == 1:
                        h0r, h0i = prev
                        rows16 = pl.ds(8 * (v - 1), 16)
                        hrr = jnp.concatenate([h0r, hr], axis=0)
                        hii = jnp.concatenate([h0i, hi], axis=0)
                        if n < 3:
                            HA[t, n, rows16, :] = hrr.astype(bf)
                            HA[t, 4 + n, rows16, :] = hii.astype(bf)
                        else:
                            HA[t, 3, rows16, :] = jnp.concatenate([hrr, hii], axis=1).astype(bf)
                    prev = (hr, hi)
                    yield

        C1 = float(np.sqrt(2.0 / np.pi))
        C2 = float(np.sqrt(2.0 / np.pi) * 0.044715)

        def s1b_chunks(t):
            for r0 in range(0, 2 * F, R1B):
                q0, q1 = r0 // 32, (r0 + R1B) // 32
                acc = nn(tobf(Wt32[q0:q1].reshape(R1B // 2, 64)), ktile(xn32, t, 3))
                for k in range(3):
                    acc = acc + nn(tobf(Wk32[k, q0:q1].reshape(R1B // 2, 128)), ktile(xn32, t, k))
                a4 = acc.reshape(R1B // 32, 2, 16, 128)
                g = a4[:, 0]
                u = a4[:, 1]
                th = jnp.tanh(g * (C1 + C2 * (g * g)))
                h2 = (g * u) * (th + 1.0)
                HB[t % 2, pl.ds(r0 // 2, R1B // 2), :] = h2.reshape(R1B // 2, 128).astype(bf)
                yield acc[ANC_ROW:ANC_ROW + 8, :]

        def s2_chunks(t):
            acc_a = None
            for k in range(7):
                d_ = nt(tobf(W2A32[k]), tobf(HA32[t, k]))
                acc_a = d_ if acc_a is None else acc_a + d_
                if k % 4 == 3:
                    yield acc_a[0:8, :]
            yield acc_a[0:8, :]
            acc_b = None
            for k0 in range(0, 14, KB):
                k1 = min(14, k0 + KB)
                wb = jnp.concatenate([tobf(W2B32[n]) for n in range(k0, k1)], axis=1)
                d_ = nn(wb, tobf(HB32[t % 2, pl.ds(64 * k0, 64 * (k1 - k0)), :]))
                acc_b = d_ if acc_b is None else acc_b + d_
                yield acc_b[0:8, :]
            x = tobf(xn32[t]).astype(f32)
            prod = (x * tabs[1]).reshape(D // 8, 8, 128)
            logit = jnp.sum(jnp.sum(prod, axis=0), axis=0, keepdims=True)
            gate = jax.nn.sigmoid(logit)
            hg = 0.5 - 0.5 * gate
            ob[t] = gate * (acc_a + x * tabs[0]) + hg * acc_b
            co[t].start()
            yield None

        def pump(gen, n):
            for _ in range(n):
                try:
                    next(gen)
                except StopIteration:
                    return False
            return True

        def chain(*gens):
            for g in gens:
                yield from g

        def transposes_steps(raw, which):
            for n in range(F // 128):
                for k in range(3):
                    v = tou(raw[pl.ds(k * 128, 128), pl.ds(n * 128, 128)].T)
                    Wk32[k, pl.ds(8 * n, 8), which] = v.reshape(8, 8, 128) | zero_u
                v = tou(raw[pl.ds(384, 64), pl.ds(n * 128, 128)].T)
                Wt32[pl.ds(8 * n, 8), which] = v.reshape(8, 8, 64) | zero_u[:, :64]
                yield

        scans = chain(*[scan_steps(t) for t in range(NT)])
        scan_done = [0]

        def pump_scan(n, anchor=None):
            if n > 0 and PACE:
                set_anchor(anchor)
            if scan_done[0] < NT * 64:
                pump(scans, n)
                scan_done[0] += n

        def ensure_scan(t, anchor=None):
            need = (t + 1) * 64 - scan_done[0]
            if need > 0:
                pump_scan(need, anchor)

        for s in range(4):
            for j in range(4 * s, 4 * s + 4):
                cx[j].wait()
            bg = None
            if s == 0:
                for c in cB:
                    c.wait()
                for c in cvec:
                    c.wait()
                build_tables()
            if s == 2:
                cwg.wait()
                bg = transposes_steps(wgr, 0)
            if s == 3:
                cwu.wait()
                bg = transposes_steps(wur, 1)
            nch = 4 * (2 * P // R1A)
            ci = 0
            for t in range(4 * s, 4 * s + 4):
                for av in s1a_chunks(t):
                    ci += 1
                    if bg is not None:
                        pump(bg, (14 * ci) // nch - (14 * (ci - 1)) // nch)
                    if s >= 1 and t - 1 >= 0:
                        lim_t = min(t - 1, P1_SCAN_TILES - 1)
                        if scan_done[0] < (lim_t + 1) * 64:
                            pump_scan(P1_SCAN_RATE, av)
            if bg is not None:
                for _ in bg:
                    pass
        for c in cC:
            c.wait()
        for c in cwd:
            c.wait()
        build_c()
        for t in range(NT):
            last = None
            for av in s1b_chunks(t):
                last = av
                lim = (min(t + LEAD, NT - 1) + 1) * 64
                pump_scan(max(0, min(P2_RATE_A, lim - scan_done[0])), av)
            ensure_scan(t, last)
            for av in s2_chunks(t):
                lim = (min(t + LEAD, NT - 1) + 1) * 64
                if av is not None:
                    pump_scan(max(0, min(P2_RATE_B, lim - scan_done[0])), av)
        for c in co:
            c.wait()

    def f(A_x, A_Lambda_re, A_Lambda_im, A_B_re, A_B_im, A_C_re, A_C_im, A_log_dt, A_Dskip, B_x, B_w_gate,
          B_w_up, B_w_down, gate_w):
        del B_x
        xT = A_x.reshape(M, D).T
        wdT = B_w_down.T
        args = [xT, A_Lambda_re, A_Lambda_im, A_B_re, A_B_im, A_C_re, A_C_im, A_log_dt, A_Dskip, B_w_gate,
                B_w_up, wdT, gate_w]
        V = pltpu.VMEM
        Hc = lambda a: pltpu.with_memory_space_constraint(a, pltpu.HBM)
        oT = pl.pallas_call(
            kernel,
            in_specs=[pl.BlockSpec(memory_space=pl.ANY)] * len(args),
            out_specs=pl.BlockSpec(memory_space=pl.ANY),
            out_shape=pltpu.HBM((D, M), f32),
            scratch_shapes=[V((D,), bf)] * 5 + [
                V((NT, D, 128), bf),
                V((3, 2 * P, 128), bf),
                V((2 * P, 64), bf),
                V((D, F), bf), V((D, F), bf),
                V((D, P), bf), V((D, P), bf),
                V((3, F // 16, 2, 8, 128), u32),
                V((F // 16, 2, 8, 64), u32),
                V((7, D, 128), bf),
                V((14, D, 128), bf),
                V((2, P, 128), f32),
                V((8, 4, 8, 128), f32),
                V((NT, 2 * P, 128), f32),
                V((NT, 7, 128, 128), bf),
                V((2, F, 128), bf),
                V((NT, D, 128), f32),
                pltpu.SemaphoreType.DMA((48,)),
                pltpu.SemaphoreType.DMA((NT,)),
            ],
            compiler_params=pltpu.CompilerParams(vmem_limit_bytes=110 * 1024 * 1024,
                                                 flags=OPT.get("flags")),
        )(*[Hc(a) for a in args])
        return oT.T.reshape(1, M, D)

    return f


_impl = make()


@jax.jit
def pallas_gated_mix__ssm_conv_s5__glu_gated_geglu__prompt_kernel(
    A_x, A_Lambda_re, A_Lambda_im, A_B_re, A_B_im, A_C_re, A_C_im, A_log_dt, A_Dskip,
    B_x, B_w_gate, B_w_up, B_w_down, gate_w,
):
    return _impl(A_x, A_Lambda_re, A_Lambda_im, A_B_re, A_B_im, A_C_re, A_C_im, A_log_dt, A_Dskip,
                 B_x, B_w_gate, B_w_up, B_w_down, gate_w)
```

```python
import jax
import jax.numpy as jnp
import numpy as np
from jax import lax
import jax.experimental.pallas as pl
import jax.experimental.pallas.tpu as pltpu

_D = 448
_P = 448
_F = 1792
_M = 2048
_NT = _M // 128

_R1A = 112
_R1B = 256
_LEAD = 2
_NQ = 4
_TQ = 4

_GELU_C1 = float(np.sqrt(2.0 / np.pi))
_GELU_C2 = float(np.sqrt(2.0 / np.pi) * 0.044715)


def _tiles(a, b, r0=0, r1=2 * _P):
    return [(t, r0, r1) for t in range(a, b)]


def _xs(a, b):
    return ["x%d" % j for j in range(a, b)]


_ORDER = ["vec"] + _xs(0, 2) + ["Bre0", "Bre1"] + _xs(2, 4) + ["Bim"] + _xs(4, 16) + ["wg", "wu", "C", "wd"]
_PLAN = [
    dict(wait=["vec"] + _xs(0, 2) + ["Bre0"], work=_tiles(0, 2, 0, 224)),
    dict(wait=["Bre1"], work=_tiles(0, 2, 224, _P)),
    dict(wait=_xs(2, 4), work=_tiles(2, 4, 0, _P)),
    dict(wait=["Bim"], work=_tiles(0, 4, _P, 2 * _P), tables=True),
    dict(wait=_xs(4, 8), work=_tiles(4, 8), scan=True),
    dict(wait=_xs(8, 16), work=_tiles(8, 13), scan=True),
    dict(wait=["wg", "wu"], work=_tiles(13, 16), scan=True, transpose=True),
]
_LATE = ["C", "wd"]


def _nn(a, b):
    return jnp.dot(a, b, preferred_element_type=jnp.float32)


def _nt(a, b):
    return lax.dot_general(a, b, (((1,), (1,)), ((), ())), preferred_element_type=jnp.float32)


def _bf16(v):
    return pltpu.bitcast(v, jnp.bfloat16)


def _u32(v):
    return pltpu.bitcast(v, jnp.uint32)


def _cmul(ar, ai, br, bi):
    return ar * br - ai * bi, ar * bi + ai * br


def _cmac(ar, ai, br, bi, cr, ci):
    return (ar * br - ai * bi) + cr, (ar * bi + ai * br) + ci


def _chain(*gens):
    for g in gens:
        yield from g


def _pump(gen, n):
    for _ in range(n):
        if next(gen, None) is None:
            return


def _kernel(xT, lre_h, lim_h, bre, bim, cre, cim, ldt_h, dsk_h, wg, wu, wdT, gw_h, o_hbm,
            lre_v, lim_v, ldt_v, dsk_v, gw_v,
            xn, Bk, Bt, wgr, wur, crr, cir, Wk32, W2A, W2B, cols, ltab, b, HA, HB, ob, sem):
    bf16, f32, u32, i32 = jnp.bfloat16, jnp.float32, jnp.uint32, jnp.int32
    D, P, F, NT = _D, _P, _F, _NT

    xn32 = xn.bitcast(u32)
    Bk32 = Bk.bitcast(u32)
    Bt32 = Bt.bitcast(u32)
    W2A32 = W2A.bitcast(u32)
    W2B32 = W2B.bitcast(u32)
    HA32 = HA.bitcast(u32)
    HB32 = HB.bitcast(u32)

    lane = lax.broadcasted_iota(i32, (8, 128), 1)
    zero_u = (lane >> 8).astype(u32)

    sem_of = {}
    for si, seg in enumerate(_PLAN):
        for name in seg["wait"]:
            sem_of[name] = si
    for name in _LATE:
        sem_of[name] = len(_PLAN)
    out_sem = len(_PLAN) + 1

    def cp(src, dst, name):
        return pltpu.make_async_copy(src, dst, sem.at[sem_of[name]])

    def b_copies(src, part, r0, r1, name):
        n, d0 = r1 - r0, part * P + r0
        cs = [cp(src.at[pl.ds(r0, n), pl.ds(k * 128, 128)], Bk.at[k, pl.ds(d0, n), :], name) for k in range(3)]
        return cs + [cp(src.at[pl.ds(r0, n), pl.ds(384, 64)], Bt.at[pl.ds(d0, n), :], name)]

    copies = {
        "vec": [cp(lre_h, lre_v, "vec"), cp(lim_h, lim_v, "vec"), cp(ldt_h, ldt_v, "vec"),
                cp(dsk_h, dsk_v, "vec"), cp(gw_h, gw_v, "vec")],
        "Bre0": b_copies(bre, 0, 0, 224, "Bre0"),
        "Bre1": b_copies(bre, 0, 224, P, "Bre1"),
        "Bim": b_copies(bim, 1, 0, P, "Bim"),
        "wg": [cp(wg, wgr, "wg")],
        "wu": [cp(wu, wur, "wu")],
        "C": [cp(cre, crr, "C"), cp(cim, cir, "C")],
        "wd": [cp(wdT.at[:, pl.ds(n * 128, 128)], W2B.at[n], "wd") for n in range(F // 128)],
    }
    for j in range(NT):
        copies["x%d" % j] = [cp(xT.at[:, pl.ds(j * 128, 128)], xn.at[j], "x%d" % j)]

    RQ = D // _NQ
    out_copies = [pltpu.make_async_copy(ob.at[j], o_hbm.at[:, pl.ds(j * 128, 128)], sem.at[out_sem])
                  for j in range(NT - 1)]
    last_copies = [pltpu.make_async_copy(ob.at[NT - 1, pl.ds(q * RQ, RQ), :],
                                         o_hbm.at[pl.ds(q * RQ, RQ), pl.ds((NT - 1) * 128, 128)], sem.at[out_sem])
                   for q in range(_NQ)]

    for name in _ORDER:
        for c in copies[name]:
            c.start()

    def wait_for(names):
        for name in names:
            for c in copies[name]:
                c.wait()

    anchor = {"bits": None}

    def set_anchor(v):
        anchor["bits"] = None if v is None else (_u32(v) & zero_u)

    def after_anchor(v):
        a = anchor["bits"]
        if a is None:
            return v
        return pltpu.bitcast(_u32(v) | a[:, :v.shape[1]], f32)

    def x_ktile(t, k):
        if k < 3:
            return _bf16(xn32[t, pl.ds(k * 64, 64), :])
        return _bf16(xn32[t, pl.ds(192, 32), :])

    def bx_rows(t, ra, rb):
        for r0 in range(ra, rb, _R1A):
            rw = pl.ds(r0 // 2, _R1A // 2)
            acc = _nn(_bf16(Bt32[rw, :]), x_ktile(t, 3))
            for k in range(3):
                acc = acc + _nn(_bf16(Bk32[k, rw, :]), x_ktile(t, k))
            b[t, pl.ds(r0, _R1A), :] = acc
            yield acc[0:8, :]

    def row(ref):
        return ref[...].astype(f32).reshape(1, D)

    def to_column(slot, v):
        for n in range(4):
            w = 128 if n < 3 else 64
            cols[slot, pl.ds(n * 128, w), :] = jnp.broadcast_to(v[:, n * 128:n * 128 + w], (128, w)).T

    coef = {}

    def build_tables():
        lr, li = row(lre_v), row(lim_v)
        dt = jnp.exp(row(ldt_v)).astype(bf16).astype(f32)
        mag = jnp.exp(dt * lr)
        lam_r, lam_i = mag * jnp.cos(dt * li), mag * jnp.sin(dt * li)
        nr, ni = lam_r - 1.0, lam_i
        big = jnp.abs(lr) >= jnp.abs(li)
        ratio = jnp.where(big, li / lr, lr / li)
        den = jnp.where(big, lr + li * ratio, lr * ratio + li)
        coef["r"] = jnp.where(big, nr + ni * ratio, nr * ratio + ni) / den
        coef["i"] = jnp.where(big, ni - nr * ratio, ni * ratio - nr) / den
        to_column(0, row(dsk_v))
        to_column(1, row(gw_v))
        p1 = (jnp.broadcast_to(lam_r, (8, D)), jnp.broadcast_to(lam_i, (8, D)))
        p2 = _cmul(*p1, *p1)
        p3 = _cmul(*p2, *p1)
        p4 = _cmul(*p2, *p2)
        pw = [p1, p2, p3, p4, _cmul(*p4, *p1), _cmul(*p4, *p2), _cmul(*p4, *p3), _cmul(*p4, *p4)]
        s8 = lax.broadcasted_iota(i32, (8, D), 0)
        l8r, l8i = pw[7]
        for s in range(7):
            l8r = jnp.where(s8 == s, pw[s][0], l8r)
            l8i = jnp.where(s8 == s, pw[s][1], l8i)
        items = [jnp.where(s8 >= 1, p1[0], 0.0), jnp.where(s8 >= 1, p1[1], 0.0),
                 jnp.where(s8 >= 2, p2[0], 0.0), jnp.where(s8 >= 2, p2[1], 0.0),
                 jnp.where(s8 >= 4, p4[0], 0.0), jnp.where(s8 >= 4, p4[1], 0.0),
                 l8r, l8i]
        for q, it in enumerate(items):
            for n in range(3):
                ltab[q, n] = it[:, n * 128:(n + 1) * 128]
            ltab[q, 3, :, pl.ds(0, 64)] = it[:, 384:448]

    def transpose_w(raw, which):
        for n in range(F // 128):
            for k in range(3):
                v = _u32(raw[pl.ds(k * 128, 128), pl.ds(n * 128, 128)].T)
                Wk32[k, pl.ds(8 * n, 8), which] = v.reshape(8, 8, 128) | zero_u
            v = _u32(raw[pl.ds(384, 64), pl.ds(n * 128, 128)].T)
            v = jnp.concatenate([v | zero_u[0:1, :64], jnp.zeros((64, 64), u32)], axis=1)
            Wk32[3, pl.ds(8 * n, 8), which] = v.reshape(8, 8, 128)
            yield True

    def build_c():
        cr2, ci2 = coef["r"] * 2.0, coef["i"] * 2.0
        for r in range(D // 16):
            if r > 0:
                yield True
            rows = pl.ds(16 * r, 16)
            for m in range(4):
                w = 128 if m < 3 else 64
                vr = crr[rows, pl.ds(m * 128, w)].astype(f32)
                vi = cir[rows, pl.ds(m * 128, w)].astype(f32)
                ar, ai = cr2[:, m * 128:m * 128 + w], ci2[:, m * 128:m * 128 + w]
                are = vr * ar - vi * ai
                aim = -(vr * ai + vi * ar)
                if m < 3:
                    W2A[m, rows, :] = are.astype(bf16)
                    W2A[4 + m, rows, :] = aim.astype(bf16)
                else:
                    W2A[3, rows, :] = jnp.concatenate([are, aim], axis=1).astype(bf16)

    carry = {}

    def scan_steps(t):
        def token_major(n):
            w = 128 if n < 3 else 64
            return b[t, pl.ds(128 * n, w), :].T, b[t, pl.ds(P + 128 * n, w), :].T

        nxt = token_major(0)
        for n in range(4):
            w = 128 if n < 3 else 64
            tre, tim = nxt
            if n < 3:
                nxt = token_major(n + 1)
            if n < 3:
                lt = [ltab[q, n] for q in range(8)]
            else:
                lt = [ltab[q, 3, :, pl.ds(0, 64)] for q in range(8)]
            prev = None
            for v in range(16):
                br = after_anchor(tre[8 * v:8 * v + 8, :])
                bi = after_anchor(tim[8 * v:8 * v + 8, :])
                for q, sh in enumerate((1, 2, 4)):
                    sr, si = pltpu.roll(br, sh, 0), pltpu.roll(bi, sh, 0)
                    br, bi = _cmac(lt[2 * q], lt[2 * q + 1], sr, si, br, bi)
                if t == 0 and v == 0:
                    hr, hi = br, bi
                else:
                    hr, hi = _cmac(lt[6], lt[7], carry[n][0], carry[n][1], br, bi)
                carry[n] = (jnp.broadcast_to(hr[7:8, :], (8, w)), jnp.broadcast_to(hi[7:8, :], (8, w)))
                if v % 2 == 1:
                    rows = pl.ds(8 * (v - 1), 16)
                    hrr = jnp.concatenate([prev[0], hr], axis=0)
                    hii = jnp.concatenate([prev[1], hi], axis=0)
                    if n < 3:
                        HA[t, n, rows, :] = hrr.astype(bf16)
                        HA[t, 4 + n, rows, :] = hii.astype(bf16)
                    else:
                        HA[t, 3, rows, :] = jnp.concatenate([hrr, hii], axis=1).astype(bf16)
                prev = (hr, hi)
                yield True

    scans = _chain(*[scan_steps(t) for t in range(NT)])
    scanned = [0]

    def pump_scan(n, anchored_to):
        n = max(0, min(n, NT * 64 - scanned[0]))
        if n > 0:
            set_anchor(anchored_to)
            _pump(scans, n)
            scanned[0] += n

    def mlp_up(t):
        xt = _bf16(jnp.concatenate([xn32[t, pl.ds(192, 32), :], jnp.zeros((32, 128), u32)], axis=0))
        for r0 in range(0, 2 * F, _R1B):
            q0, q1 = r0 // 32, (r0 + _R1B) // 32
            acc = _nn(_bf16(Wk32[3, q0:q1].reshape(_R1B // 2, 128)), xt)
            for k in range(3):
                acc = acc + _nn(_bf16(Wk32[k, q0:q1].reshape(_R1B // 2, 128)), x_ktile(t, k))
            a4 = acc.reshape(_R1B // 32, 2, 16, 128)
            g, u = a4[:, 0], a4[:, 1]
            th = jnp.tanh(g * (_GELU_C1 + _GELU_C2 * (g * g)))
            h2 = (g * u) * (th + 1.0)
            HB[t % 2, pl.ds(r0 // 2, _R1B // 2), :] = h2.reshape(_R1B // 2, 128).astype(bf16)
            yield acc[0:8, :]

    def gate_of(t):
        x = _bf16(xn32[t]).astype(f32)
        prod = (x * cols[1]).reshape(D // 8, 8, 128)
        gate = jax.nn.sigmoid(jnp.sum(jnp.sum(prod, axis=0), axis=0, keepdims=True))
        return x, gate, 0.5 - 0.5 * gate

    def hb_tile(t, k):
        return _bf16(HB32[t % 2, pl.ds(64 * k, 64), :])

    def project(t, mlp_first=False, background=None):
        accs = {}

        def ssm_part():
            acc = None
            for k in range(7):
                d = _nt(_bf16(W2A32[k]), _bf16(HA32[t, k]))
                acc = d if acc is None else acc + d
                accs["a"] = acc
                if k % 4 == 3:
                    yield acc[0:8, :]
            yield acc[0:8, :]

        def mlp_part():
            acc = None
            for k in range(F // 128):
                if k == F // 128 - 1:
                    d = jnp.concatenate([_nn(_bf16(W2B32[k, pl.ds(56 * q, 56), :]), hb_tile(t, k))
                                         for q in range(4)], axis=0)
                else:
                    d = _nn(_bf16(W2B32[k]), hb_tile(t, k))
                acc = d if acc is None else acc + d
                accs["b"] = acc
                if background is not None:
                    _pump(background, 3)
                if k % 4 == 3 or k == F // 128 - 1:
                    yield acc[0:8, :]

        if mlp_first:
            yield from mlp_part()
            for _ in background:
                pass
            yield from ssm_part()
        else:
            yield from ssm_part()
            yield from mlp_part()
        x, gate, hg = gate_of(t)
        ob[t] = gate * (accs["a"] + x * cols[0]) + hg * accs["b"]
        out_copies[t].start()

    def project_last(t):
        x, gate, hg = gate_of(t)
        acc_a = None
        for k in range(7):
            d = _nt(_bf16(W2A32[k]), _bf16(HA32[t, k]))
            acc_a = d if acc_a is None else acc_a + d
        acc_b = None
        for k in range(F // 128 - _TQ):
            d = _nn(_bf16(W2B32[k]), hb_tile(t, k))
            acc_b = d if acc_b is None else acc_b + d
        base = gate * (acc_a + x * cols[0])
        base = base + hg * acc_b
        for q in range(_NQ):
            acc = None
            for k in range(F // 128 - _TQ, F // 128):
                d = _nn(_bf16(W2B32[k, pl.ds(q * RQ // 2, RQ // 2), :]), hb_tile(t, k))
                acc = d if acc is None else acc + d
            ob[t, pl.ds(q * RQ, RQ), :] = base[q * RQ:(q + 1) * RQ] + hg * acc
            last_copies[q].start()

    for seg in _PLAN:
        wait_for(seg["wait"])
        if seg.get("tables"):
            build_tables()
        bg = _chain(transpose_w(wgr, 0), transpose_w(wur, 1)) if seg.get("transpose") else None
        nch = sum((r1 - r0) // _R1A for _, r0, r1 in seg["work"])
        ci = 0
        for t, ra, rb in seg["work"]:
            for last in bx_rows(t, ra, rb):
                ci += 1
                if bg is not None:
                    _pump(bg, (2 * (F // 128) * ci) // nch - (2 * (F // 128) * (ci - 1)) // nch)
                if seg.get("scan") and scanned[0] < (_LEAD + 1) * 64 and ci < nch:
                    pump_scan(min(3, (_LEAD + 1) * 64 - scanned[0]), last)
        if bg is not None:
            for _ in bg:
                pass

    for t in range(NT):
        limit = (min(t + _LEAD, NT - 1) + 1) * 64
        last = None
        for last in mlp_up(t):
            pump_scan(min(3, limit - scanned[0]), last)
        pump_scan((t + 1) * 64 - scanned[0], last)
        if t == NT - 1:
            project_last(t)
            continue
        background = None
        if t == 0:
            wait_for(_LATE)
            background = build_c()
        for last in project(t, mlp_first=(t == 0), background=background):
            pump_scan(min(4, limit - scanned[0]), last)

    for c in out_copies + last_copies:
        c.wait()


@jax.jit
def pallas_gated_mix__ssm_conv_s5__glu_gated_geglu__prompt_kernel(
    A_x, A_Lambda_re, A_Lambda_im, A_B_re, A_B_im, A_C_re, A_C_im, A_log_dt, A_Dskip,
    B_x, B_w_gate, B_w_up, B_w_down, gate_w,
):
    del B_x
    bf16, f32, u32 = jnp.bfloat16, jnp.float32, jnp.uint32
    D, P, F, M, NT = _D, _P, _F, _M, _NT
    args = [A_x.reshape(M, D).T, A_Lambda_re, A_Lambda_im, A_B_re, A_B_im, A_C_re, A_C_im, A_log_dt, A_Dskip,
            B_w_gate, B_w_up, B_w_down.T, gate_w]
    V = pltpu.VMEM
    out_t = pl.pallas_call(
        _kernel,
        in_specs=[pl.BlockSpec(memory_space=pl.ANY)] * len(args),
        out_specs=pl.BlockSpec(memory_space=pl.ANY),
        out_shape=pltpu.HBM((D, M), f32),
        scratch_shapes=[V((D,), bf16)] * 5 + [
            V((NT, D, 128), bf16),
            V((3, 2 * P, 128), bf16),
            V((2 * P, 64), bf16),
            V((D, F), bf16), V((D, F), bf16),
            V((D, P), bf16), V((D, P), bf16),
            V((4, F // 16, 2, 8, 128), u32),
            V((7, D, 128), bf16),
            V((F // 128, D, 128), bf16),
            V((2, D, 128), f32),
            V((8, 4, 8, 128), f32),
            V((NT, 2 * P, 128), f32),
            V((NT, 7, 128, 128), bf16),
            V((2, F, 128), bf16),
            V((NT, D, 128), f32),
            pltpu.SemaphoreType.DMA((len(_PLAN) + 2,)),
        ],
        compiler_params=pltpu.CompilerParams(vmem_limit_bytes=110 * 1024 * 1024),
    )(*[pltpu.with_memory_space_constraint(a, pltpu.HBM) for a in args])
    return out_t.T.reshape(1, M, D)
```

```python
import jax
import jax.numpy as jnp
import numpy as np
from jax import lax
import jax.experimental.pallas as pl
import jax.experimental.pallas.tpu as pltpu

_D = 448
_P = 448
_F = 1792
_M = 2048
_NT = _M // 128

_R1A = 112
_R1B = 256
_LEAD = 2
_NQ = 4
_TQ = 4

_GELU_C1 = float(np.sqrt(2.0 / np.pi))
_GELU_C2 = float(np.sqrt(2.0 / np.pi) * 0.044715)


def _tiles(a, b, r0=0, r1=2 * _P):
    return [(t, r0, r1) for t in range(a, b)]


def _xs(a, b):
    return ["x%d" % j for j in range(a, b)]


_ORDER = ["vec"] + _xs(0, 2) + ["Bre0", "Bre1"] + _xs(2, 4) + ["Bim"] + _xs(4, 16) + ["wg", "wu", "C", "wd"]
_PLAN = [
    dict(wait=["vec"] + _xs(0, 2) + ["Bre0"], work=_tiles(0, 2, 0, 224)),
    dict(wait=["Bre1"], work=_tiles(0, 2, 224, _P)),
    dict(wait=_xs(2, 4), work=_tiles(2, 4, 0, _P)),
    dict(wait=["Bim"], work=_tiles(0, 4, _P, 2 * _P), tables=True),
    dict(wait=_xs(4, 8), work=_tiles(4, 8), scan=True),
    dict(wait=_xs(8, 16), work=_tiles(8, 13), scan=True),
    dict(wait=["wg", "wu"], work=_tiles(13, 16), scan=True, transpose=True),
]
_LATE = ["C", "wd"]


def _nn(a, b):
    return jnp.dot(a, b, preferred_element_type=jnp.float32)


def _nt(a, b):
    return lax.dot_general(a, b, (((1,), (1,)), ((), ())), preferred_element_type=jnp.float32)


def _bf16(v):
    return pltpu.bitcast(v, jnp.bfloat16)


def _u32(v):
    return pltpu.bitcast(v, jnp.uint32)


def _cmul(ar, ai, br, bi):
    return ar * br - ai * bi, ar * bi + ai * br


def _cmac(ar, ai, br, bi, cr, ci):
    return (ar * br - ai * bi) + cr, (ar * bi + ai * br) + ci


def _chain(*gens):
    for g in gens:
        yield from g


def _pump(gen, n):
    for _ in range(n):
        if next(gen, None) is None:
            return


def _kernel(xT, lre_h, lim_h, bre, bim, cre, cim, ldt_h, dsk_h, wg, wu, wdT, gw_h, o_hbm,
            lre_v, lim_v, ldt_v, dsk_v, gw_v,
            xn, Bk, Bt, wgr, wur, crr, cir, Wk32, W2A, W2B, cols, ltab, b, HA, HB, ob, sem):
    bf16, f32, u32, i32 = jnp.bfloat16, jnp.float32, jnp.uint32, jnp.int32
    D, P, F, NT = _D, _P, _F, _NT

    xn32 = xn.bitcast(u32)
    Bk32 = Bk.bitcast(u32)
    Bt32 = Bt.bitcast(u32)
    W2A32 = W2A.bitcast(u32)
    W2B32 = W2B.bitcast(u32)
    HA32 = HA.bitcast(u32)
    HB32 = HB.bitcast(u32)

    lane = lax.broadcasted_iota(i32, (8, 128), 1)
    zero_u = (lane >> 8).astype(u32)

    sem_of = {}
    for si, seg in enumerate(_PLAN):
        for name in seg["wait"]:
            sem_of[name] = si
    for name in _LATE:
        sem_of[name] = len(_PLAN)
    out_sem = len(_PLAN) + 1

    def cp(src, dst, name):
        return pltpu.make_async_copy(src, dst, sem.at[sem_of[name]])

    def b_copies(src, part, r0, r1, name):
        n, d0 = r1 - r0, part * P + r0
        cs = [cp(src.at[pl.ds(r0, n), pl.ds(k * 128, 128)], Bk.at[k, pl.ds(d0, n), :], name) for k in range(3)]
        return cs + [cp(src.at[pl.ds(r0, n), pl.ds(384, 64)], Bt.at[pl.ds(d0, n), :], name)]

    copies = {
        "vec": [cp(lre_h, lre_v, "vec"), cp(lim_h, lim_v, "vec"), cp(ldt_h, ldt_v, "vec"),
                cp(dsk_h, dsk_v, "vec"), cp(gw_h, gw_v, "vec")],
        "Bre0": b_copies(bre, 0, 0, 224, "Bre0"),
        "Bre1": b_copies(bre, 0, 224, P, "Bre1"),
        "Bim": b_copies(bim, 1, 0, P, "Bim"),
        "wg": [cp(wg, wgr, "wg")],
        "wu": [cp(wu, wur, "wu")],
        "C": [cp(cre, crr, "C"), cp(cim, cir, "C")],
        "wd": [cp(wdT.at[:, pl.ds(n * 128, 128)], W2B.at[n], "wd") for n in range(F // 128)],
    }
    for j in range(NT):
        copies["x%d" % j] = [cp(xT.at[:, pl.ds(j * 128, 128)], xn.at[j], "x%d" % j)]

    RQ = D // _NQ
    out_copies = [pltpu.make_async_copy(ob.at[j], o_hbm.at[:, pl.ds(j * 128, 128)], sem.at[out_sem])
                  for j in range(NT - 1)]
    last_copies = [pltpu.make_async_copy(ob.at[NT - 1, pl.ds(q * RQ, RQ), :],
                                         o_hbm.at[pl.ds(q * RQ, RQ), pl.ds((NT - 1) * 128, 128)], sem.at[out_sem])
                   for q in range(_NQ)]

    for name in _ORDER:
        for c in copies[name]:
            c.start()

    def wait_for(names):
        for name in names:
            for c in copies[name]:
                c.wait()

    anchor = {"bits": None}

    def set_anchor(v):
        anchor["bits"] = None if v is None else (_u32(v) & zero_u)

    def after_anchor(v):
        a = anchor["bits"]
        if a is None:
            return v
        return pltpu.bitcast(_u32(v) | a[:, :v.shape[1]], f32)

    def x_ktile(t, k):
        if k < 3:
            return _bf16(xn32[t, pl.ds(k * 64, 64), :])
        return _bf16(xn32[t, pl.ds(192, 32), :])

    def bx_rows(t, ra, rb):
        for r0 in range(ra, rb, _R1A):
            rw = pl.ds(r0 // 2, _R1A // 2)
            acc = _nn(_bf16(Bt32[rw, :]), x_ktile(t, 3))
            for k in range(3):
                acc = acc + _nn(_bf16(Bk32[k, rw, :]), x_ktile(t, k))
            b[t, pl.ds(r0, _R1A), :] = acc
            yield acc[0:8, :]

    def row(ref):
        return ref[...].astype(f32).reshape(1, D)

    def to_column(slot, v):
        for n in range(4):
            w = 128 if n < 3 else 64
            cols[slot, pl.ds(n * 128, w), :] = jnp.broadcast_to(v[:, n * 128:n * 128 + w], (128, w)).T

    coef = {}

    def build_tables():
        lr, li = row(lre_v), row(lim_v)
        dt = jnp.exp(row(ldt_v)).astype(bf16).astype(f32)
        mag = jnp.exp(dt * lr)
        lam_r, lam_i = mag * jnp.cos(dt * li), mag * jnp.sin(dt * li)
        nr, ni = lam_r - 1.0, lam_i
        big = jnp.abs(lr) >= jnp.abs(li)
        ratio = jnp.where(big, li / lr, lr / li)
        den = jnp.where(big, lr + li * ratio, lr * ratio + li)
        coef["r"] = jnp.where(big, nr + ni * ratio, nr * ratio + ni) / den
        coef["i"] = jnp.where(big, ni - nr * ratio, ni * ratio - nr) / den
        to_column(0, row(dsk_v))
        to_column(1, row(gw_v))
        p1 = (jnp.broadcast_to(lam_r, (8, D)), jnp.broadcast_to(lam_i, (8, D)))
        p2 = _cmul(*p1, *p1)
        p3 = _cmul(*p2, *p1)
        p4 = _cmul(*p2, *p2)
        pw = [p1, p2, p3, p4, _cmul(*p4, *p1), _cmul(*p4, *p2), _cmul(*p4, *p3), _cmul(*p4, *p4)]
        s8 = lax.broadcasted_iota(i32, (8, D), 0)
        l8r, l8i = pw[7]
        for s in range(7):
            l8r = jnp.where(s8 == s, pw[s][0], l8r)
            l8i = jnp.where(s8 == s, pw[s][1], l8i)
        items = [jnp.where(s8 >= 1, p1[0], 0.0), jnp.where(s8 >= 1, p1[1], 0.0),
                 jnp.where(s8 >= 2, p2[0], 0.0), jnp.where(s8 >= 2, p2[1], 0.0),
                 jnp.where(s8 >= 4, p4[0], 0.0), jnp.where(s8 >= 4, p4[1], 0.0),
                 l8r, l8i]
        for q, it in enumerate(items):
            for n in range(3):
                ltab[q, n] = it[:, n * 128:(n + 1) * 128]
            ltab[q, 3, :, pl.ds(0, 64)] = it[:, 384:448]

    def transpose_w(raw, which):
        for n in range(F // 128):
            for k in range(3):
                v = _u32(raw[pl.ds(k * 128, 128), pl.ds(n * 128, 128)].T)
                Wk32[k, pl.ds(8 * n, 8), which] = v.reshape(8, 8, 128) | zero_u
            v = _u32(raw[pl.ds(384, 64), pl.ds(n * 128, 128)].T)
            v = jnp.concatenate([v | zero_u[0:1, :64], jnp.zeros((64, 64), u32)], axis=1)
            Wk32[3, pl.ds(8 * n, 8), which] = v.reshape(8, 8, 128)
            yield True

    def build_c():
        cr2, ci2 = coef["r"] * 2.0, coef["i"] * 2.0
        for r in range(D // 16):
            if r > 0:
                yield True
            rows = pl.ds(16 * r, 16)
            for m in range(4):
                w = 128 if m < 3 else 64
                vr = crr[rows, pl.ds(m * 128, w)].astype(f32)
                vi = cir[rows, pl.ds(m * 128, w)].astype(f32)
                ar, ai = cr2[:, m * 128:m * 128 + w], ci2[:, m * 128:m * 128 + w]
                are = vr * ar - vi * ai
                aim = -(vr * ai + vi * ar)
                if m < 3:
                    W2A[m, rows, :] = are.astype(bf16)
                    W2A[4 + m, rows, :] = aim.astype(bf16)
                else:
                    W2A[3, rows, :] = jnp.concatenate([are, aim], axis=1).astype(bf16)

    carry = {}

    def scan_steps(t):
        def token_major(n):
            w = 128 if n < 3 else 64
            return b[t, pl.ds(128 * n, w), :].T, b[t, pl.ds(P + 128 * n, w), :].T

        nxt = token_major(0)
        for n in range(4):
            w = 128 if n < 3 else 64
            tre, tim = nxt
            if n < 3:
                nxt = token_major(n + 1)
            if n < 3:
                lt = [ltab[q, n] for q in range(8)]
            else:
                lt = [ltab[q, 3, :, pl.ds(0, 64)] for q in range(8)]
            prev = None
            for v in range(16):
                br = after_anchor(tre[8 * v:8 * v + 8, :])
                bi = after_anchor(tim[8 * v:8 * v + 8, :])
                for q, sh in enumerate((1, 2, 4)):
                    sr, si = pltpu.roll(br, sh, 0), pltpu.roll(bi, sh, 0)
                    br, bi = _cmac(lt[2 * q], lt[2 * q + 1], sr, si, br, bi)
                if t == 0 and v == 0:
                    hr, hi = br, bi
                else:
                    hr, hi = _cmac(lt[6], lt[7], carry[n][0], carry[n][1], br, bi)
                carry[n] = (jnp.broadcast_to(hr[7:8, :], (8, w)), jnp.broadcast_to(hi[7:8, :], (8, w)))
                if v % 2 == 1:
                    rows = pl.ds(8 * (v - 1), 16)
                    hrr = jnp.concatenate([prev[0], hr], axis=0)
                    hii = jnp.concatenate([prev[1], hi], axis=0)
                    if n < 3:
                        HA[t, n, rows, :] = hrr.astype(bf16)
                        HA[t, 4 + n, rows, :] = hii.astype(bf16)
                    else:
                        HA[t, 3, rows, :] = jnp.concatenate([hrr, hii], axis=1).astype(bf16)
                prev = (hr, hi)
                yield True

    scans = _chain(*[scan_steps(t) for t in range(NT)])
    scanned = [0]

    def pump_scan(n, anchored_to):
        n = max(0, min(n, NT * 64 - scanned[0]))
        if n > 0:
            set_anchor(anchored_to)
            _pump(scans, n)
            scanned[0] += n

    def mlp_up(t):
        xt = _bf16(jnp.concatenate([xn32[t, pl.ds(192, 32), :], jnp.zeros((32, 128), u32)], axis=0))
        for r0 in range(0, 2 * F, _R1B):
            q0, q1 = r0 // 32, (r0 + _R1B) // 32
            acc = _nn(_bf16(Wk32[3, q0:q1].reshape(_R1B // 2, 128)), xt)
            for k in range(3):
                acc = acc + _nn(_bf16(Wk32[k, q0:q1].reshape(_R1B // 2, 128)), x_ktile(t, k))
            a4 = acc.reshape(_R1B // 32, 2, 16, 128)
            g, u = a4[:, 0], a4[:, 1]
            th = jnp.tanh(g * (_GELU_C1 + _GELU_C2 * (g * g)))
            h2 = (g * u) * (th + 1.0)
            HB[t % 2, pl.ds(r0 // 2, _R1B // 2), :] = h2.reshape(_R1B // 2, 128).astype(bf16)
            yield acc[0:8, :]

    def gate_of(t):
        x = _bf16(xn32[t]).astype(f32)
        prod = (x * cols[1]).reshape(D // 8, 8, 128)
        gate = jax.nn.sigmoid(jnp.sum(jnp.sum(prod, axis=0), axis=0, keepdims=True))
        return x, gate, 0.5 - 0.5 * gate

    def hb_tile(t, k):
        return _bf16(HB32[t % 2, pl.ds(64 * k, 64), :])

    def project(t, mlp_first=False, background=None):
        accs = {}

        def ssm_part():
            acc = None
            for k in range(7):
                d = _nt(_bf16(W2A32[k]), _bf16(HA32[t, k]))
                acc = d if acc is None else acc + d
                accs["a"] = acc
                if k % 4 == 3:
                    yield acc[0:8, :]
            yield acc[0:8, :]

        def mlp_part():
            acc = None
            for k in range(F // 128):
                if k == F // 128 - 1:
                    d = jnp.concatenate([_nn(_bf16(W2B32[k, pl.ds(56 * q, 56), :]), hb_tile(t, k))
                                         for q in range(4)], axis=0)
                else:
                    d = _nn(_bf16(W2B32[k]), hb_tile(t, k))
                acc = d if acc is None else acc + d
                accs["b"] = acc
                if background is not None:
                    _pump(background, 3)
                if k % 4 == 3 or k == F // 128 - 1:
                    yield acc[0:8, :]

        if mlp_first:
            yield from mlp_part()
            for _ in background:
                pass
            yield from ssm_part()
        else:
            yield from ssm_part()
            yield from mlp_part()
        x, gate, hg = gate_of(t)
        ob[t] = gate * (accs["a"] + x * cols[0]) + hg * accs["b"]
        out_copies[t].start()

    def project_last(t):
        x, gate, hg = gate_of(t)
        acc_a = None
        for k in range(7):
            d = _nt(_bf16(W2A32[k]), _bf16(HA32[t, k]))
            acc_a = d if acc_a is None else acc_a + d
        acc_b = None
        for k in range(F // 128 - _TQ):
            d = _nn(_bf16(W2B32[k]), hb_tile(t, k))
            acc_b = d if acc_b is None else acc_b + d
        base = gate * (acc_a + x * cols[0])
        base = base + hg * acc_b
        for q in range(_NQ):
            acc = None
            for k in range(F // 128 - _TQ, F // 128):
                d = _nn(_bf16(W2B32[k, pl.ds(q * RQ // 2, RQ // 2), :]), hb_tile(t, k))
                acc = d if acc is None else acc + d
            ob[t, pl.ds(q * RQ, RQ), :] = base[q * RQ:(q + 1) * RQ] + hg * acc
            last_copies[q].start()

    for seg in _PLAN:
        wait_for(seg["wait"])
        if seg.get("tables"):
            build_tables()
        bg = _chain(transpose_w(wgr, 0), transpose_w(wur, 1)) if seg.get("transpose") else None
        nch = sum((r1 - r0) // _R1A for _, r0, r1 in seg["work"])
        ci = 0
        for t, ra, rb in seg["work"]:
            for last in bx_rows(t, ra, rb):
                ci += 1
                if bg is not None:
                    _pump(bg, (2 * (F // 128) * ci) // nch - (2 * (F // 128) * (ci - 1)) // nch)
                if seg.get("scan") and scanned[0] < (_LEAD + 1) * 64 and ci < nch:
                    pump_scan(min(3, (_LEAD + 1) * 64 - scanned[0]), last)
        if bg is not None:
            for _ in bg:
                pass

    for t in range(NT):
        limit = (min(t + _LEAD, NT - 1) + 1) * 64
        last = None
        for last in mlp_up(t):
            pump_scan(min(3, limit - scanned[0]), last)
        pump_scan((t + 1) * 64 - scanned[0], last)
        if t == NT - 1:
            project_last(t)
            continue
        background = None
        if t == 0:
            wait_for(_LATE)
            background = build_c()
        for last in project(t, mlp_first=(t == 0), background=background):
            pump_scan(min(4, limit - scanned[0]), last)

    for c in out_copies + last_copies:
        c.wait()


@jax.jit
def pallas_gated_mix__ssm_conv_s5__glu_gated_geglu__prompt_kernel(
    A_x, A_Lambda_re, A_Lambda_im, A_B_re, A_B_im, A_C_re, A_C_im, A_log_dt, A_Dskip,
    B_x, B_w_gate, B_w_up, B_w_down, gate_w,
):
    del B_x
    bf16, f32, u32 = jnp.bfloat16, jnp.float32, jnp.uint32
    D, P, F, M, NT = _D, _P, _F, _M, _NT
    args = [A_x.reshape(M, D).T, A_Lambda_re, A_Lambda_im, A_B_re, A_B_im, A_C_re, A_C_im, A_log_dt, A_Dskip,
            B_w_gate, B_w_up, B_w_down.T, gate_w]
    V = pltpu.VMEM
    out_t = pl.pallas_call(
        _kernel,
        in_specs=[pl.BlockSpec(memory_space=pltpu.HBM)] * len(args),
        out_specs=pl.BlockSpec(memory_space=pltpu.HBM),
        out_shape=jax.ShapeDtypeStruct((D, M), f32),
        scratch_shapes=[V((D,), bf16)] * 5 + [
            V((NT, D, 128), bf16),
            V((3, 2 * P, 128), bf16),
            V((2 * P, 64), bf16),
            V((D, F), bf16), V((D, F), bf16),
            V((D, P), bf16), V((D, P), bf16),
            V((4, F // 16, 2, 8, 128), u32),
            V((7, D, 128), bf16),
            V((F // 128, D, 128), bf16),
            V((2, D, 128), f32),
            V((8, 4, 8, 128), f32),
            V((NT, 2 * P, 128), f32),
            V((NT, 7, 128, 128), bf16),
            V((2, F, 128), bf16),
            V((NT, D, 128), f32),
            pltpu.SemaphoreType.DMA((len(_PLAN) + 2,)),
        ],
        compiler_params=pltpu.CompilerParams(vmem_limit_bytes=110 * 1024 * 1024),
    )(*args)
    return out_t.T.reshape(1, M, D)
```

```python
import jax
import jax.numpy as jnp
import numpy as np
from jax import lax
import jax.experimental.pallas as pl
import jax.experimental.pallas.tpu as pltpu

_D = 448
_P = 448
_F = 1792
_M = 2048
_NT = _M // 128

_R1A = 112
_R1B = 256
_LEAD = 2
_NQ = 4
_TQ = 4

_GELU_C1 = float(np.sqrt(2.0 / np.pi))
_GELU_C2 = float(np.sqrt(2.0 / np.pi) * 0.044715)


def _tiles(a, b, r0=0, r1=2 * _P):
    return [(t, r0, r1) for t in range(a, b)]


def _xs(a, b):
    return ["x%d" % j for j in range(a, b)]


_ORDER = ["vec"] + _xs(0, 2) + ["Bre0", "Bre1"] + _xs(2, 4) + ["Bim"] + _xs(4, 16) + ["wg", "wu", "C", "wd"]
_PLAN = [
    dict(wait=["vec"] + _xs(0, 2) + ["Bre0"], work=_tiles(0, 2, 0, 224)),
    dict(wait=["Bre1"], work=_tiles(0, 2, 224, _P)),
    dict(wait=_xs(2, 4), work=_tiles(2, 4, 0, _P)),
    dict(wait=["Bim"], work=_tiles(0, 4, _P, 2 * _P), tables=True),
    dict(wait=_xs(4, 8), work=_tiles(4, 8), scan=True),
    dict(wait=_xs(8, 16), work=_tiles(8, 13), scan=True),
    dict(wait=["wg", "wu"], work=_tiles(13, 16), scan=True, transpose=True),
]
_XGROUP = [(0, 0), (0, 1), (1, 0), (1, 1)] + [(2, j) for j in range(4)] + [(3, j) for j in range(8)]
_LATE = ["C", "wd"]


def _nn(a, b):
    return jnp.dot(a, b, preferred_element_type=jnp.float32)


def _nt(a, b):
    return lax.dot_general(a, b, (((1,), (1,)), ((), ())), preferred_element_type=jnp.float32)


def _bf16(v):
    return pltpu.bitcast(v, jnp.bfloat16)


def _u32(v):
    return pltpu.bitcast(v, jnp.uint32)


def _cmul(ar, ai, br, bi):
    return ar * br - ai * bi, ar * bi + ai * br


def _cmac(ar, ai, br, bi, cr, ci):
    return (ar * br - ai * bi) + cr, (ar * bi + ai * br) + ci


def _chain(*gens):
    for g in gens:
        yield from g


def _pump(gen, n):
    for _ in range(n):
        if next(gen, None) is None:
            return


def _kernel(xT, lre_h, lim_h, bre, bim, cre, cim, ldt_h, dsk_h, wg, wu, wdT, gw_h, o_hbm,
            lre_v, lim_v, ldt_v, dsk_v, gw_v,
            xn0, xn1, xn2, xn3, Bk0, Bk1, Bk2, Bt0, Bt1, Bt2,
            wgr, wur, crr, cir, Wk32, W2A, W2B, cols, ltab, b, HA, HB, ob, sem):
    bf16, f32, u32, i32 = jnp.bfloat16, jnp.float32, jnp.uint32, jnp.int32
    D, P, F, NT = _D, _P, _F, _NT

    xn = [(xn0, xn1, xn2, xn3)[g].at[j] for g, j in _XGROUP]
    xn32 = [(xn0, xn1, xn2, xn3)[g].bitcast(u32).at[j] for g, j in _XGROUP]
    Bk, Bt = (Bk0, Bk1, Bk2), (Bt0, Bt1, Bt2)
    Bk32 = [r.bitcast(u32) for r in Bk]
    Bt32 = [r.bitcast(u32) for r in Bt]
    W2A32 = W2A.bitcast(u32)
    W2B32 = W2B.bitcast(u32)
    HA32 = HA.bitcast(u32)
    HB32 = HB.bitcast(u32)

    lane = lax.broadcasted_iota(i32, (8, 128), 1)
    zero_u = (lane >> 8).astype(u32)

    sem_of = {}
    for si, seg in enumerate(_PLAN):
        for name in seg["wait"]:
            sem_of[name] = si
    for name in _LATE:
        sem_of[name] = len(_PLAN)
    out_sem = len(_PLAN) + 1

    def cp(src, dst, name):
        return pltpu.make_async_copy(src, dst, sem.at[sem_of[name]])

    def b_copies(src, r0, r1, part, name):
        rows = pl.ds(r0, r1 - r0)
        cs = [cp(src.at[rows, pl.ds(k * 128, 128)], Bk[part].at[k], name) for k in range(3)]
        return cs + [cp(src.at[rows, pl.ds(384, 64)], Bt[part], name)]

    copies = {
        "vec": [cp(lre_h, lre_v, "vec"), cp(lim_h, lim_v, "vec"), cp(ldt_h, ldt_v, "vec"),
                cp(dsk_h, dsk_v, "vec"), cp(gw_h, gw_v, "vec")],
        "Bre0": b_copies(bre, 0, 224, 0, "Bre0"),
        "Bre1": b_copies(bre, 224, P, 1, "Bre1"),
        "Bim": b_copies(bim, 0, P, 2, "Bim"),
        "wg": [cp(wg, wgr, "wg")],
        "wu": [cp(wu, wur, "wu")],
        "C": [cp(cre, crr, "C"), cp(cim, cir, "C")],
        "wd": [cp(wdT.at[:, pl.ds(n * 128, 128)], W2B.at[n], "wd") for n in range(F // 128)],
    }
    for j in range(NT):
        copies["x%d" % j] = [cp(xT.at[:, pl.ds(j * 128, 128)], xn[j], "x%d" % j)]

    RQ = D // _NQ
    out_copies = [pltpu.make_async_copy(ob.at[j], o_hbm.at[:, pl.ds(j * 128, 128)], sem.at[out_sem])
                  for j in range(NT - 1)]
    last_copies = [pltpu.make_async_copy(ob.at[NT - 1, pl.ds(q * RQ, RQ), :],
                                         o_hbm.at[pl.ds(q * RQ, RQ), pl.ds((NT - 1) * 128, 128)], sem.at[out_sem])
                   for q in range(_NQ)]

    for name in _ORDER:
        for c in copies[name]:
            c.start()

    def wait_for(names):
        for name in names:
            for c in copies[name]:
                c.wait()

    anchor = {"bits": None}

    def set_anchor(v):
        anchor["bits"] = None if v is None else (_u32(v) & zero_u)

    def after_anchor(v):
        a = anchor["bits"]
        if a is None:
            return v
        return pltpu.bitcast(_u32(v) | a[:, :v.shape[1]], f32)

    def x_ktile(t, k):
        if k < 3:
            return _bf16(xn32[t][pl.ds(k * 64, 64), :])
        return _bf16(xn32[t][pl.ds(192, 32), :])

    def bx_rows(t, ra, rb):
        for r0 in range(ra, rb, _R1A):
            part = 0 if r0 < 224 else (1 if r0 < P else 2)
            rw = pl.ds((r0 - (0, 224, P)[part]) // 2, _R1A // 2)
            acc = _nn(_bf16(Bt32[part][rw, :]), x_ktile(t, 3))
            for k in range(3):
                acc = acc + _nn(_bf16(Bk32[part][k, rw, :]), x_ktile(t, k))
            b[t, pl.ds(r0, _R1A), :] = acc
            yield acc[0:8, :]

    def row(ref):
        return ref[...].astype(f32).reshape(1, D)

    def to_column(slot, v):
        for n in range(4):
            w = 128 if n < 3 else 64
            cols[slot, pl.ds(n * 128, w), :] = jnp.broadcast_to(v[:, n * 128:n * 128 + w], (128, w)).T

    coef = {}

    def build_tables():
        lr, li = row(lre_v), row(lim_v)
        dt = jnp.exp(row(ldt_v)).astype(bf16).astype(f32)
        mag = jnp.exp(dt * lr)
        lam_r, lam_i = mag * jnp.cos(dt * li), mag * jnp.sin(dt * li)
        nr, ni = lam_r - 1.0, lam_i
        big = jnp.abs(lr) >= jnp.abs(li)
        ratio = jnp.where(big, li / lr, lr / li)
        den = jnp.where(big, lr + li * ratio, lr * ratio + li)
        coef["r"] = jnp.where(big, nr + ni * ratio, nr * ratio + ni) / den
        coef["i"] = jnp.where(big, ni - nr * ratio, ni * ratio - nr) / den
        to_column(0, row(dsk_v))
        to_column(1, row(gw_v))
        p1 = (jnp.broadcast_to(lam_r, (8, D)), jnp.broadcast_to(lam_i, (8, D)))
        p2 = _cmul(*p1, *p1)
        p3 = _cmul(*p2, *p1)
        p4 = _cmul(*p2, *p2)
        pw = [p1, p2, p3, p4, _cmul(*p4, *p1), _cmul(*p4, *p2), _cmul(*p4, *p3), _cmul(*p4, *p4)]
        s8 = lax.broadcasted_iota(i32, (8, D), 0)
        l8r, l8i = pw[7]
        for s in range(7):
            l8r = jnp.where(s8 == s, pw[s][0], l8r)
            l8i = jnp.where(s8 == s, pw[s][1], l8i)
        items = [jnp.where(s8 >= 1, p1[0], 0.0), jnp.where(s8 >= 1, p1[1], 0.0),
                 jnp.where(s8 >= 2, p2[0], 0.0), jnp.where(s8 >= 2, p2[1], 0.0),
                 jnp.where(s8 >= 4, p4[0], 0.0), jnp.where(s8 >= 4, p4[1], 0.0),
                 l8r, l8i]
        for q, it in enumerate(items):
            for n in range(3):
                ltab[q, n] = it[:, n * 128:(n + 1) * 128]
            ltab[q, 3, :, pl.ds(0, 64)] = it[:, 384:448]

    def transpose_w(raw, which):
        for n in range(F // 128):
            for k in range(3):
                v = _u32(raw[pl.ds(k * 128, 128), pl.ds(n * 128, 128)].T)
                Wk32[k, pl.ds(8 * n, 8), which] = v.reshape(8, 8, 128) | zero_u
            v = _u32(raw[pl.ds(384, 64), pl.ds(n * 128, 128)].T)
            v = jnp.concatenate([v | zero_u[0:1, :64], jnp.zeros((64, 64), u32)], axis=1)
            Wk32[3, pl.ds(8 * n, 8), which] = v.reshape(8, 8, 128)
            yield True

    def build_c():
        cr2, ci2 = coef["r"] * 2.0, coef["i"] * 2.0
        for r in range(D // 16):
            if r > 0:
                yield True
            rows = pl.ds(16 * r, 16)
            for m in range(4):
                w = 128 if m < 3 else 64
                vr = crr[rows, pl.ds(m * 128, w)].astype(f32)
                vi = cir[rows, pl.ds(m * 128, w)].astype(f32)
                ar, ai = cr2[:, m * 128:m * 128 + w], ci2[:, m * 128:m * 128 + w]
                are = vr * ar - vi * ai
                aim = -(vr * ai + vi * ar)
                if m < 3:
                    W2A[m, rows, :] = are.astype(bf16)
                    W2A[4 + m, rows, :] = aim.astype(bf16)
                else:
                    W2A[3, rows, :] = jnp.concatenate([are, aim], axis=1).astype(bf16)

    carry = {}

    def scan_steps(t):
        def token_major(n):
            w = 128 if n < 3 else 64
            return b[t, pl.ds(128 * n, w), :].T, b[t, pl.ds(P + 128 * n, w), :].T

        nxt = token_major(0)
        for n in range(4):
            w = 128 if n < 3 else 64
            tre, tim = nxt
            if n < 3:
                nxt = token_major(n + 1)
            if n < 3:
                lt = [ltab[q, n] for q in range(8)]
            else:
                lt = [ltab[q, 3, :, pl.ds(0, 64)] for q in range(8)]
            prev = None
            for v in range(16):
                br = after_anchor(tre[8 * v:8 * v + 8, :])
                bi = after_anchor(tim[8 * v:8 * v + 8, :])
                for q, sh in enumerate((1, 2, 4)):
                    sr, si = pltpu.roll(br, sh, 0), pltpu.roll(bi, sh, 0)
                    br, bi = _cmac(lt[2 * q], lt[2 * q + 1], sr, si, br, bi)
                if t == 0 and v == 0:
                    hr, hi = br, bi
                else:
                    hr, hi = _cmac(lt[6], lt[7], carry[n][0], carry[n][1], br, bi)
                carry[n] = (jnp.broadcast_to(hr[7:8, :], (8, w)), jnp.broadcast_to(hi[7:8, :], (8, w)))
                if v % 2 == 1:
                    rows = pl.ds(8 * (v - 1), 16)
                    hrr = jnp.concatenate([prev[0], hr], axis=0)
                    hii = jnp.concatenate([prev[1], hi], axis=0)
                    if n < 3:
                        HA[t, n, rows, :] = hrr.astype(bf16)
                        HA[t, 4 + n, rows, :] = hii.astype(bf16)
                    else:
                        HA[t, 3, rows, :] = jnp.concatenate([hrr, hii], axis=1).astype(bf16)
                prev = (hr, hi)
                yield True

    scans = _chain(*[scan_steps(t) for t in range(NT)])
    scanned = [0]

    def pump_scan(n, anchored_to):
        n = max(0, min(n, NT * 64 - scanned[0]))
        if n > 0:
            set_anchor(anchored_to)
            _pump(scans, n)
            scanned[0] += n

    def mlp_up(t):
        xt = _bf16(jnp.concatenate([xn32[t][pl.ds(192, 32), :], jnp.zeros((32, 128), u32)], axis=0))
        for r0 in range(0, 2 * F, _R1B):
            q0, q1 = r0 // 32, (r0 + _R1B) // 32
            acc = _nn(_bf16(Wk32[3, q0:q1].reshape(_R1B // 2, 128)), xt)
            for k in range(3):
                acc = acc + _nn(_bf16(Wk32[k, q0:q1].reshape(_R1B // 2, 128)), x_ktile(t, k))
            a4 = acc.reshape(_R1B // 32, 2, 16, 128)
            g, u = a4[:, 0], a4[:, 1]
            th = jnp.tanh(g * (_GELU_C1 + _GELU_C2 * (g * g)))
            h2 = (g * u) * (th + 1.0)
            HB[t % 2, pl.ds(r0 // 2, _R1B // 2), :] = h2.reshape(_R1B // 2, 128).astype(bf16)
            yield acc[0:8, :]

    def gate_of(t):
        x = _bf16(xn32[t][...]).astype(f32)
        prod = (x * cols[1]).reshape(D // 8, 8, 128)
        gate = jax.nn.sigmoid(jnp.sum(jnp.sum(prod, axis=0), axis=0, keepdims=True))
        return x, gate, 0.5 - 0.5 * gate

    def hb_tile(t, k):
        return _bf16(HB32[t % 2, pl.ds(64 * k, 64), :])

    def project(t, mlp_first=False, background=None):
        accs = {}

        def ssm_part():
            acc = None
            for k in range(7):
                d = _nt(_bf16(W2A32[k]), _bf16(HA32[t, k]))
                acc = d if acc is None else acc + d
                accs["a"] = acc
                if k % 4 == 3:
                    yield acc[0:8, :]
            yield acc[0:8, :]

        def mlp_part():
            acc = None
            for k in range(F // 128):
                if k == F // 128 - 1:
                    d = jnp.concatenate([_nn(_bf16(W2B32[k, pl.ds(56 * q, 56), :]), hb_tile(t, k))
                                         for q in range(4)], axis=0)
                else:
                    d = _nn(_bf16(W2B32[k]), hb_tile(t, k))
                acc = d if acc is None else acc + d
                accs["b"] = acc
                if background is not None:
                    _pump(background, 3)
                if k % 4 == 3 or k == F // 128 - 1:
                    yield acc[0:8, :]

        if mlp_first:
            yield from mlp_part()
            for _ in background:
                pass
            yield from ssm_part()
        else:
            yield from ssm_part()
            yield from mlp_part()
        x, gate, hg = gate_of(t)
        ob[t] = gate * (accs["a"] + x * cols[0]) + hg * accs["b"]
        out_copies[t].start()

    def project_last(t):
        x, gate, hg = gate_of(t)
        acc_a = None
        for k in range(7):
            d = _nt(_bf16(W2A32[k]), _bf16(HA32[t, k]))
            acc_a = d if acc_a is None else acc_a + d
        acc_b = None
        for k in range(F // 128 - _TQ):
            d = _nn(_bf16(W2B32[k]), hb_tile(t, k))
            acc_b = d if acc_b is None else acc_b + d
        base = gate * (acc_a + x * cols[0])
        base = base + hg * acc_b
        for q in range(_NQ):
            acc = None
            for k in range(F // 128 - _TQ, F // 128):
                d = _nn(_bf16(W2B32[k, pl.ds(q * RQ // 2, RQ // 2), :]), hb_tile(t, k))
                acc = d if acc is None else acc + d
            ob[t, pl.ds(q * RQ, RQ), :] = base[q * RQ:(q + 1) * RQ] + hg * acc
            last_copies[q].start()

    for seg in _PLAN:
        wait_for(seg["wait"])
        if seg.get("tables"):
            build_tables()
        bg = _chain(transpose_w(wgr, 0), transpose_w(wur, 1)) if seg.get("transpose") else None
        nch = sum((r1 - r0) // _R1A for _, r0, r1 in seg["work"])
        ci = 0
        for t, ra, rb in seg["work"]:
            for last in bx_rows(t, ra, rb):
                ci += 1
                if bg is not None:
                    _pump(bg, (2 * (F // 128) * ci) // nch - (2 * (F // 128) * (ci - 1)) // nch)
                if seg.get("scan") and scanned[0] < (_LEAD + 1) * 64 and ci < nch:
                    pump_scan(min(3, (_LEAD + 1) * 64 - scanned[0]), last)
        if bg is not None:
            for _ in bg:
                pass

    for t in range(NT):
        limit = (min(t + _LEAD, NT - 1) + 1) * 64
        last = None
        for last in mlp_up(t):
            pump_scan(min(3, limit - scanned[0]), last)
        pump_scan((t + 1) * 64 - scanned[0], last)
        if t == NT - 1:
            project_last(t)
            continue
        background = None
        if t == 0:
            wait_for(_LATE)
            background = build_c()
        for last in project(t, mlp_first=(t == 0), background=background):
            pump_scan(min(4, limit - scanned[0]), last)

    for c in out_copies + last_copies:
        c.wait()


@jax.jit
def pallas_gated_mix__ssm_conv_s5__glu_gated_geglu__prompt_kernel(
    A_x, A_Lambda_re, A_Lambda_im, A_B_re, A_B_im, A_C_re, A_C_im, A_log_dt, A_Dskip,
    B_x, B_w_gate, B_w_up, B_w_down, gate_w,
):
    del B_x
    bf16, f32, u32 = jnp.bfloat16, jnp.float32, jnp.uint32
    D, P, F, M, NT = _D, _P, _F, _M, _NT
    args = [A_x.reshape(M, D).T, A_Lambda_re, A_Lambda_im, A_B_re, A_B_im, A_C_re, A_C_im, A_log_dt, A_Dskip,
            B_w_gate, B_w_up, B_w_down.T, gate_w]
    V = pltpu.VMEM
    out_t = pl.pallas_call(
        _kernel,
        in_specs=[pl.BlockSpec(memory_space=pltpu.HBM)] * len(args),
        out_specs=pl.BlockSpec(memory_space=pltpu.HBM),
        out_shape=jax.ShapeDtypeStruct((D, M), f32),
        scratch_shapes=[V((D,), bf16)] * 5 + [
            V((2, D, 128), bf16), V((2, D, 128), bf16),
            V((4, D, 128), bf16), V((8, D, 128), bf16),
            V((3, 224, 128), bf16), V((3, 224, 128), bf16),
            V((3, P, 128), bf16),
            V((224, 64), bf16), V((224, 64), bf16),
            V((P, 64), bf16),
            V((D, F), bf16), V((D, F), bf16),
            V((D, P), bf16), V((D, P), bf16),
            V((4, F // 16, 2, 8, 128), u32),
            V((7, D, 128), bf16),
            V((F // 128, D, 128), bf16),
            V((2, D, 128), f32),
            V((8, 4, 8, 128), f32),
            V((NT, 2 * P, 128), f32),
            V((NT, 7, 128, 128), bf16),
            V((2, F, 128), bf16),
            V((NT, D, 128), f32),
            pltpu.SemaphoreType.DMA((len(_PLAN) + 2,)),
        ],
        compiler_params=pltpu.CompilerParams(vmem_limit_bytes=110 * 1024 * 1024),
    )(*args)
    return out_t.T.reshape(1, M, D)
```
